```python
import os as _os
_os.environ.setdefault("JAX_PLATFORMS", "cpu")
import jax
import jax.numpy as jnp

def _softmax(x, axis=-1):
    return jax.nn.softmax(x, axis=axis)
def _gelu(x):
    return jax.nn.gelu(x, approximate=True)
def _silu(x):
    return jax.nn.silu(x)
def _sigmoid(x):
    return jax.nn.sigmoid(x)
def _layernorm(x, axis=-1, eps=1e-5):
    m = jnp.mean(x, axis=axis, keepdims=True)
    v = jnp.var(x, axis=axis, keepdims=True)
    return (x - m) / jnp.sqrt(v + eps)
def _scatter_add(tgt, idx, src, axis=0):
    return tgt.at[idx].add(src)
def _segment_sum(src, seg, n):
    return jax.ops.segment_sum(src, seg, n)
class _Rng:
    def __init__(self, key):
        self._k = key
    def _next(self):
        self._k, sub = jax.random.split(self._k)
        return sub
    def normal(self, shape):
        return jax.random.normal(self._next(), shape, dtype=jnp.bfloat16)
    def randint(self, lo, hi, shape):
        return jax.random.randint(self._next(), shape, lo, hi, dtype=jnp.int32)
    def uniform(self, shape, lo=0.0, hi=1.0):
        return jax.random.uniform(self._next(), shape, jnp.bfloat16, lo, hi)
    def permutation(self, n):
        return jax.random.permutation(self._next(), n)


kernel_name = 'concat_heads__mha_block_cached__gqa_block_cached__decode'

def setup_inputs():
    _rng = _Rng(jax.random.key(int.from_bytes(__import__("os").urandom(4), "little")))
    _w = (lambda a: (lambda t: t.astype(jnp.bfloat16) if jnp.issubdtype(t.dtype, jnp.floating) else t)(jnp.asarray(a)))
    def _A_setup():
        B, Sq, D = 1, 1, 512
        H, Sk, Dh = 32, 4096, 128
        return {
            "x": _w((lambda *s: _rng.normal(s) * 0.8)(B, Sq, D)),
            "k_cache": _w((lambda *s: _rng.normal(s) * 0.8)(B, H, Sk, Dh)),
            "v_cache": _w((lambda *s: _rng.normal(s) * 0.05)(B, H, Sk, Dh)),
            "wq": _w((lambda *s: _rng.normal(s) * 0.8)(D, H * Dh) * (D ** -0.5)),
            "wo": _w((lambda *s: _rng.normal(s) * 0.05)(H * Dh, D) * ((H * Dh) ** -0.5)),
        }
    _A_in = _A_setup()

    def _B_setup():
        B, Sq, D = 1, 1, 512
        Hq, Hkv, Sk, Dh = 32, 32, 4096, 128
        assert Hq % Hkv == 0, (Hq, Hkv)
        return {
            "x": _w((lambda *s: _rng.normal(s) * 0.8)(B, Sq, D)),
            "k_cache": _w((lambda *s: _rng.normal(s) * 0.8)(B, Hkv, Sk, Dh)),
            "v_cache": _w((lambda *s: _rng.normal(s) * 0.05)(B, Hkv, Sk, Dh)),
            "wq": _w((lambda *s: _rng.normal(s) * 0.8)(D, Hq * Dh) * (D ** -0.5)),
            "wo": _w((lambda *s: _rng.normal(s) * 0.05)(Hq * Dh, D) * ((Hq * Dh) ** -0.5)),
        }
    _B_in = _B_setup()

    return {
        "A_x": _A_in["x"],
        "A_k_cache": _A_in["k_cache"],
        "A_v_cache": _A_in["v_cache"],
        "A_wq": _A_in["wq"],
        "A_wo": _A_in["wo"],
        "B_x": _B_in["x"],
        "B_k_cache": _B_in["k_cache"],
        "B_v_cache": _B_in["v_cache"],
        "B_wq": _B_in["wq"],
        "B_wo": _B_in["wo"],
    }

def reference(A_x, A_k_cache, A_v_cache, A_wq, A_wo, B_x, B_k_cache, B_v_cache, B_wq, B_wo):
    def _A_ref(x, k_cache, v_cache, wq, wo):
        B, Sq, D = x.shape
        H, Dh = 32, 128
        q = (lambda x, *d: x.transpose(*d))((x @ wq).reshape(B, Sq, H, Dh), 0, 2, 1, 3)
        scores = jnp.einsum("bhqd,bhkd->bhqk", q, k_cache) * (Dh ** -0.5)
        p = _softmax(scores, axis=-1)
        o = jnp.einsum("bhqk,bhkd->bhqd", p, v_cache)
        return (lambda x, *d: x.transpose(*d))(o, 0, 2, 1, 3).reshape(B, Sq, H * Dh) @ wo

    def _B_ref(x, k_cache, v_cache, wq, wo):
        B, Sq, D = x.shape
        Hq, Dh = 32, 128
        Hkv = k_cache.shape[1]
        rep = Hq // Hkv
        q = (lambda x, *d: x.transpose(*d))((x @ wq).reshape(B, Sq, Hq, Dh), 0, 2, 1, 3)
        k = jnp.repeat(k_cache, rep, axis=1)
        v = jnp.repeat(v_cache, rep, axis=1)
        scores = jnp.einsum("bhqd,bhkd->bhqk", q, k) * (Dh ** -0.5)
        p = _softmax(scores, axis=-1)
        o = jnp.einsum("bhqk,bhkd->bhqd", p, v)
        return (lambda x, *d: x.transpose(*d))(o, 0, 2, 1, 3).reshape(B, Sq, Hq * Dh) @ wo

    a = _A_ref(A_x, A_k_cache, A_v_cache, A_wq, A_wo)
    b = _B_ref(B_x, B_k_cache, B_v_cache, B_wq, B_wo)
    return jnp.concatenate([a, b], axis=-1)
```

```python
import functools
import numpy as np
import jax
import jax.numpy as jnp
from jax import lax
from jax.experimental import pallas as pl
from jax.experimental.pallas import tpu as pltpu

D, H, S, DH = 512, 32, 4096, 128
G = 8
NG = H // G
RB = 16
F32, BF16 = jnp.float32, jnp.bfloat16


def build(KB=512, LAG=2, SLOTS=4, issue_unroll=4, compute=True, nochk=True):
    NKB = S // KB
    NDMA = KB // RB
    NSTEP = NG * NKB
    NW = 128 // NDMA

    def kern(ax, ak, av, awq, awo, bx, bk, bv, bwq, bwo, o_ref,
             xbuf, wqb, wob, ring, q_scr, s_scr, m_scr, l_scr, acc_scr, o_scr, sems, wsem):
        row = lax.broadcasted_iota(jnp.int32, (G, DH), 0)

        def issue_wq(t):
            @pl.loop(0, NDMA, unroll=issue_unroll)
            def _(i):
                n = t * NDMA + i
                r = pl.multiple_of((n // 32) * RB, RB)
                c = pl.multiple_of((n % 32) * 128, 128)
                for j, w in enumerate((awq, bwq)):
                    pltpu.make_async_copy(w.at[:, pl.ds(r, RB), pl.ds(c, 128)],
                                          wqb.at[j, :, pl.ds(r, RB), pl.ds(c, 128)],
                                          wsem.at[0]).start(priority=j)

        def issue_wo(t):
            @pl.loop(0, NDMA, unroll=issue_unroll)
            def _(i):
                n = t * NDMA + i
                r = pl.multiple_of((n // 4) * RB, RB)
                c = pl.multiple_of((n % 4) * 128, 128)
                for j, w in enumerate((awo, bwo)):
                    pltpu.make_async_copy(w.at[:, pl.ds(r, RB), pl.ds(c, 128)],
                                          wob.at[j, :, pl.ds(r, RB), pl.ds(c, 128)],
                                          wsem.at[1]).start(priority=j)

        def issue_kv(srcs, t, base):
            slot = (t + base) % SLOTS
            h0 = pl.multiple_of((t // NKB) * G, G)
            k0 = (t % NKB) * KB
            @pl.loop(0, NDMA, unroll=issue_unroll)
            def _(i):
                r = pl.multiple_of(i * RB, RB)
                for j, a in enumerate(srcs):
                    pltpu.make_async_copy(a.at[0, pl.ds(h0, G), pl.ds(pl.multiple_of(k0 + r, RB), RB)],
                                          ring.at[slot, j, :, pl.ds(r, RB)],
                                          sems.at[slot]).start(priority=j)

        def wait_slot(slot):
            pltpu.make_async_copy(ring.at[slot], ring.at[slot], sems.at[slot]).wait()

        def q_group(g):
            for j in range(2):
                x8 = jnp.broadcast_to(xbuf[j, 0], (G, D))
                c0 = pl.multiple_of(g * (G * DH), G * DH)
                w = wqb[j, :, :, pl.ds(c0, G * DH)].reshape(D, G * DH)
                r = jnp.dot(x8, w, preferred_element_type=F32)
                q = r[:, :DH]
                for h in range(1, G):
                    q = jnp.where(row == h, r[:, h * DH:(h + 1) * DH], q)
                q_scr[j, g] = q

        def k_step(t):
            slot = t % SLOTS
            g = t // NKB
            kb = t % NKB
            wait_slot(slot)
            if not compute:
                return
            rowk = lax.broadcasted_iota(jnp.int32, (G, KB), 0)
            for j in range(2):
                q = q_scr[j, g].astype(BF16)
                s = None
                for h in range(G):
                    r = lax.dot_general(q, ring[slot, j, h], (((1,), (1,)), ((), ())),
                                        preferred_element_type=F32)
                    s = r if s is None else jnp.where(rowk == h, r, s)
                s = s * (DH ** -0.5)
                s_scr[j, g, kb] = s
                m = s[:, :DH]
                for c in range(1, KB // DH):
                    m = jnp.maximum(m, s[:, c * DH:(c + 1) * DH])
                m_scr[j, g] = jnp.maximum(m_scr[j, g], m)

        def v_step(t):
            slot = (t + NSTEP) % SLOTS
            g = t // NKB
            kb = t % NKB
            wait_slot(slot)
            if not compute:
                return
            for j in range(2):
                m = jnp.max(m_scr[j, g], axis=-1, keepdims=True)
                p = jnp.exp(s_scr[j, g, kb] - m)
                l = p[:, :DH]
                for c in range(1, KB // DH):
                    l = l + p[:, c * DH:(c + 1) * DH]
                l_scr[j, g] += l
                pb = p.astype(BF16)
                o = None
                for h in range(G):
                    r = jnp.dot(pb, ring[slot, j, h], preferred_element_type=F32)
                    o = r if o is None else jnp.where(row == h, r, o)
                acc_scr[j, g] += o

        issue_wq(0)
        xc = [pltpu.make_async_copy(x, xbuf.at[j], wsem.at[2 + j]) for j, x in enumerate((ax, bx))]
        for c in xc:
            c.start()
        m_scr[...] = jnp.full(m_scr.shape, -jnp.inf, F32)
        l_scr[...] = jnp.zeros(l_scr.shape, F32)
        acc_scr[...] = jnp.zeros(acc_scr.shape, F32)

        @pl.loop(1, NW)
        def _(t):
            issue_wq(t)
        @pl.loop(0, LAG)
        def _(t):
            issue_kv((ak, bk), t, 0)
        for c in xc:
            c.wait()
        pltpu.make_async_copy(wqb, wqb, wsem.at[0]).wait()

        @pl.loop(0, NSTEP)
        def _(t):
            if compute:
                @pl.when(t % NKB == 0)
                def _():
                    q_group(t // NKB)
            @pl.when(t + LAG < NSTEP)
            def _():
                issue_kv((ak, bk), t + LAG, 0)
            @pl.when(t + LAG >= NSTEP)
            def _():
                issue_kv((av, bv), t + LAG - NSTEP, NSTEP)
            k_step(t)

        @pl.loop(0, NSTEP)
        def _(t):
            @pl.when(t + LAG < NSTEP)
            def _():
                issue_kv((av, bv), t + LAG, NSTEP)
            @pl.when(t + LAG >= NSTEP)
            def _():
                issue_wo(t + LAG - NSTEP)
            v_step(t)

        @pl.loop(LAG, NW)
        def _(t):
            issue_wo(t)

        for j in range(2):
            for g in range(NG):
                l = jnp.sum(l_scr[j, g], axis=-1, keepdims=True)
                o = acc_scr[j, g] / l
                for h in range(G):
                    o_scr[j, :, pl.ds((g * G + h) * DH, DH)] = jnp.broadcast_to(o[h:h + 1], (G, DH))
        pltpu.make_async_copy(wob, wob, wsem.at[1]).wait()
        for j in range(2):
            if compute:
                r = jnp.dot(o_scr[j].astype(BF16), wob[j].reshape(H * DH, D), preferred_element_type=F32)
            else:
                r = jnp.zeros((8, D), F32)
            o_ref[0, :, pl.ds(j * D, D)] = r[0:1].astype(o_ref.dtype)

    def f(A_x, A_k, A_v, A_wq, A_wo, B_x, B_k, B_v, B_wq, B_wo):
        return pl.pallas_call(
            kern,
            out_shape=jax.ShapeDtypeStruct((1, 1, 2 * D), BF16),
            in_specs=[pl.BlockSpec(memory_space=pl.ANY)] * 10,
            out_specs=pl.BlockSpec(memory_space=pltpu.VMEM),
            scratch_shapes=[
                pltpu.VMEM((2, 1, 1, D), BF16),
                pltpu.VMEM((2, 8, D // 8, H * DH), BF16),
                pltpu.VMEM((2, 8, H * DH // 8, D), BF16),
                pltpu.VMEM((SLOTS, 2, G, KB, DH), BF16),
                pltpu.VMEM((2, NG, G, DH), F32),
                pltpu.VMEM((2, NG, NKB, G, KB), F32),
                pltpu.VMEM((2, NG, G, DH), F32),
                pltpu.VMEM((2, NG, G, DH), F32),
                pltpu.VMEM((2, NG, G, DH), F32),
                pltpu.VMEM((2, G, H * DH), F32),
                pltpu.SemaphoreType.DMA((SLOTS,)),
                pltpu.SemaphoreType.DMA((4,)),
            ],
            compiler_params=pltpu.CompilerParams(
                vmem_limit_bytes=100 * 1024 * 1024,
                disable_semaphore_checks=nochk, disable_bounds_checks=nochk),
        )(A_x, A_k, A_v, A_wq.reshape(8, D // 8, H * DH), A_wo.reshape(8, H * DH // 8, D),
          B_x, B_k, B_v, B_wq.reshape(8, D // 8, H * DH), B_wo.reshape(8, H * DH // 8, D))
    return f


@jax.jit
def pallas_concat_heads__mha_block_cached__gqa_block_cached__decode_kernel(
    A_x, A_k_cache, A_v_cache, A_wq, A_wo, B_x, B_k_cache, B_v_cache, B_wq, B_wo,
):
    return build(KB=256, LAG=4, SLOTS=8)(
        A_x, A_k_cache, A_v_cache, A_wq, A_wo, B_x, B_k_cache, B_v_cache, B_wq, B_wo)
```

```python
import jax
import jax.numpy as jnp
from jax import lax
import jax.experimental.pallas as pl
import jax.experimental.pallas.tpu as pltpu

D, H, S, DH = 512, 32, 4096, 128
G = 8
NG = 2 * H // G
GH = 2 * G
KB = 512
NKB = S // KB
NS = (H // GH) * NKB
SLOTS, LAG = 4, 2
WQ = 4
KV_UNIT = 32
KV_COPIES = ((0, 6, 0, 32, 1), (11, 5, 0, 16, 0), (6, 5, 0, 32, 1), (11, 5, 16, 16, 0))
TAIL = ((0, 5), (5, 7), (7, 8))


def _log2(n):
    assert n & (n - 1) == 0
    return n.bit_length() - 1


def _wait_all(view, sem):
    pltpu.make_async_copy(view, view, sem).wait()


def _lane_tiles(x):
    return [x[:, c:c + DH] for c in range(0, x.shape[1], DH)]


def _own_rows(parts):
    row = lax.broadcasted_iota(jnp.int32, parts[0].shape, 0)
    out = parts[0]
    for h in range(1, len(parts)):
        out = jnp.where(row == h, parts[h], out)
    return out


def _kernel(ax, ak, av, awq, awo, bx, bk, bv, bwq, bwo, o_ref,
            x_buf, wq_buf, wo_buf, ring, q_scr, s_scr, m_scr, l_scr, acc_scr, out_scr,
            ring_sem, w_sem, tail_sem):
    dtype = ring.dtype

    def start_weights(lo, hi):
        @pl.loop(lo, hi, unroll=2)
        def _(n):
            rows = pl.ds(pl.multiple_of((n >> 3) << 3, 8), 8)
            cols = pl.ds(pl.multiple_of((n & 7) * D, D), D)
            for j, w in enumerate((awq, bwq)):
                pltpu.make_async_copy(
                    w.at[:, rows, cols], wq_buf.at[j, :, rows, cols], w_sem.at[0]
                ).start(priority=1)
            rows = pl.ds(pl.multiple_of(n << 3, 8), 8)
            for j, w in enumerate((awo, bwo)):
                pltpu.make_async_copy(
                    w.at[pl.ds(0, WQ - j), rows],
                    wo_buf.at[pl.ds(WQ * j, WQ - j), rows],
                    w_sem.at[1],
                ).start(priority=1 - j)

    def start_tail():
        for k, (lo, hi) in enumerate(TAIL):
            for h in range(lo, hi):
                rows = pl.ds(h * DH, DH)
                pltpu.make_async_copy(
                    bwo.at[WQ - 1, rows], wo_buf.at[NG - 1, rows], tail_sem.at[k]
                ).start(priority=1)

    def start_step(cache, t):
        slot = t & (SLOTS - 1)
        head0 = (t >> _log2(NKB)) * GH
        key0 = (t & (NKB - 1)) * KB

        @pl.loop(0, KB // KV_UNIT, unroll=2)
        def _(i):
            for head, heads, key, keys, priority in KV_COPIES:
                r = i * KV_UNIT + key
                pltpu.make_async_copy(
                    cache.at[0, pl.ds(head0 + head, heads),
                             pl.ds(pl.multiple_of(key0 + r, keys), keys)],
                    ring.at[slot, pl.ds(head, heads), pl.ds(pl.multiple_of(r, keys), keys)],
                    ring_sem.at[slot],
                ).start(priority=priority)

    def start_ahead(t, caches):
        n = t + LAG
        for i, cache in enumerate(caches):
            @pl.when((n >> _log2(NS)) == i)
            def _():
                start_step(cache, n & (NS - 1))

    def project_q(t):
        j = t >> _log2(NS)
        g0 = ((t & (NS - 1)) >> _log2(NKB)) * 2
        x = jnp.broadcast_to(x_buf[j, 0], (G, D))
        for u in range(2):
            cols = pl.ds(pl.multiple_of((g0 + u) * (G * DH), G * DH), G * DH)
            w = wq_buf[j, :, :, cols].reshape(D, G * DH)
            q = jnp.dot(x, w, preferred_element_type=jnp.float32)
            q_scr[u] = _own_rows(_lane_tiles(q))

    def scores(t):
        slot = t & (SLOTS - 1)
        g0 = (t >> _log2(NKB)) * 2
        _wait_all(ring.at[slot], ring_sem.at[slot])
        for u in range(2):
            q = q_scr[u].astype(dtype)
            s = _own_rows([
                lax.dot_general(q, ring[slot, u * G + h], (((1,), (1,)), ((), ())),
                                preferred_element_type=jnp.float32)
                for h in range(G)
            ]) * (DH ** -0.5)
            s_scr[t, u] = s
            m = m_scr[g0 + u]
            for tile in _lane_tiles(s):
                m = jnp.maximum(m, tile)
            m_scr[g0 + u] = m

    def values(t):
        slot = t & (SLOTS - 1)
        g0 = (t >> _log2(NKB)) * 2
        probs = []
        for u in range(2):
            row_max = jnp.max(m_scr[g0 + u], axis=-1, keepdims=True)
            p = jnp.exp(s_scr[t, u] - row_max)
            l = l_scr[g0 + u]
            for tile in _lane_tiles(p):
                l = l + tile
            l_scr[g0 + u] = l
            probs.append(p.astype(dtype))
        _wait_all(ring.at[slot], ring_sem.at[slot])
        for u in range(2):
            acc_scr[g0 + u] += _own_rows([
                jnp.dot(probs[u], ring[slot, u * G + h], preferred_element_type=jnp.float32)
                for h in range(G)
            ])

    def head_outputs(g):
        o = acc_scr[g] / jnp.sum(l_scr[g], axis=-1, keepdims=True)
        return [jnp.broadcast_to(o[h:h + 1], (G, DH)).astype(dtype) for h in range(G)]

    start_weights(0, 8)
    x_copies = [pltpu.make_async_copy(x, x_buf.at[j], w_sem.at[2 + j])
                for j, x in enumerate((ax, bx))]
    for c in x_copies:
        c.start()
    m_scr[...] = jnp.full(m_scr.shape, -jnp.inf, jnp.float32)
    l_scr[...] = jnp.zeros(l_scr.shape, jnp.float32)
    acc_scr[...] = jnp.zeros(acc_scr.shape, jnp.float32)
    out_scr[...] = jnp.zeros(out_scr.shape, jnp.float32)
    start_weights(8, G * DH // 8)

    @pl.loop(0, LAG)
    def _(t):
        start_step(ak, t)

    for c in x_copies:
        c.wait()
    _wait_all(wq_buf, w_sem.at[0])
    _wait_all(wo_buf.at[pl.ds(0, NG - 1)], w_sem.at[1])

    @pl.loop(0, 2 * NS)
    def _(t):
        @pl.when((t & (NKB - 1)) == 0)
        def _():
            project_q(t)

        start_ahead(t, (ak, bk, av))
        scores(t)

    @pl.loop(0, 2 * NS)
    def _(t):
        start_ahead(t, (av, bv))
        pl.when(t + LAG == 2 * NS)(start_tail)
        values(t)

        @pl.when(jnp.logical_and(((t + 1) & (NKB - 1)) < 2, t > 0))
        def _():
            g = 2 * (((t + 1) >> _log2(NKB)) - 1) + ((t + 1) & 1)
            out_scr[g >> _log2(NG // 2)] += jnp.dot(
                jnp.concatenate(head_outputs(g), axis=1), wo_buf[g],
                preferred_element_type=jnp.float32)

    o_ref[0, :, pl.ds(0, D)] = out_scr[0, 0:1].astype(o_ref.dtype)
    heads = head_outputs(NG - 1)
    out = out_scr[1]
    for k, (lo, hi) in enumerate(TAIL):
        rows = pl.ds(lo * DH, (hi - lo) * DH)
        _wait_all(wo_buf.at[NG - 1, rows], tail_sem.at[k])
        out += jnp.dot(jnp.concatenate(heads[lo:hi], axis=1), wo_buf[NG - 1, rows],
                       preferred_element_type=jnp.float32)
    o_ref[0, :, pl.ds(D, D)] = out[0:1].astype(o_ref.dtype)


@jax.jit
def pallas_concat_heads__mha_block_cached__gqa_block_cached__decode_kernel(
    A_x: jax.Array,
    A_k_cache: jax.Array,
    A_v_cache: jax.Array,
    A_wq: jax.Array,
    A_wo: jax.Array,
    B_x: jax.Array,
    B_k_cache: jax.Array,
    B_v_cache: jax.Array,
    B_wq: jax.Array,
    B_wo: jax.Array,
):
    for cache in (A_k_cache, A_v_cache, B_k_cache, B_v_cache):
        assert cache.shape == (1, H, S, DH), cache.shape
    dtype = A_k_cache.dtype
    split_wq = lambda w: w.reshape(WQ, D // WQ, H * DH)
    split_wo = lambda w: w.reshape(WQ, H * DH // WQ, D)

    return pl.pallas_call(
        _kernel,
        out_shape=jax.ShapeDtypeStruct((1, 1, 2 * D), A_x.dtype),
        in_specs=[pl.BlockSpec(memory_space=pl.ANY)] * 10,
        out_specs=pl.BlockSpec(memory_space=pltpu.VMEM),
        scratch_shapes=[
            pltpu.VMEM((2, 1, 1, D), dtype),
            pltpu.VMEM((2, WQ, D // WQ, H * DH), dtype),
            pltpu.VMEM((NG, G * DH, D), dtype),
            pltpu.VMEM((SLOTS, GH, KB, DH), dtype),
            pltpu.VMEM((2, G, DH), jnp.float32),
            pltpu.VMEM((2 * NS, 2, G, KB), jnp.float32),
            pltpu.VMEM((NG, G, DH), jnp.float32),
            pltpu.VMEM((NG, G, DH), jnp.float32),
            pltpu.VMEM((NG, G, DH), jnp.float32),
            pltpu.VMEM((2, G, D), jnp.float32),
            pltpu.SemaphoreType.DMA((SLOTS,)),
            pltpu.SemaphoreType.DMA((4,)),
            pltpu.SemaphoreType.DMA((len(TAIL),)),
        ],
        compiler_params=pltpu.CompilerParams(
            vmem_limit_bytes=48 * 1024 * 1024,
            disable_semaphore_checks=True,
        ),
    )(A_x, A_k_cache, A_v_cache, split_wq(A_wq), split_wo(A_wo),
      B_x, B_k_cache, B_v_cache, split_wq(B_wq), split_wo(B_wo))
```

```python
import jax
import jax.numpy as jnp
from jax import lax
import jax.experimental.pallas as pl
import jax.experimental.pallas.tpu as pltpu

D, H, S, DH = 512, 32, 4096, 128
G = 8
NG = 2 * H // G
GH = 2 * G
KB = 256
NKB = S // KB
NS = (H // GH) * NKB
SLOTS, LAG = 4, 3

KV_KEYS = 64
KV_COPIES = ((0, 1), (2, 1), (10, 0), (4, 1), (6, 1), (12, 0), (8, 1), (14, 0))
WQ = 4
WQ_ROWS, WQ_COLS, WO_ROWS = 8, 1024, 16
W_ROUNDS = G * DH // WO_ROWS
W_COPIES = (("wo", 0, 0, 2, 1), ("wq", 0, 0, 1, 0), ("wo", 0, 2, 2, 1), ("wq", 0, 1, 1, 0),
            ("wq", 1, 0, 2, 1), ("wq", 1, 2, 2, 1), ("wq", 0, 2, 1, 0), ("wo", 1, 0, 3, 1),
            ("wq", 0, 3, 1, 0))
TAIL = ((0, 640), (640, 768), (768, 896), (896, 992), (992, 1024))


def _log2(n):
    assert n & (n - 1) == 0
    return n.bit_length() - 1


def _block(i, size):
    return pl.ds(pl.multiple_of(i * size, size), size)


def _wait_all(view, sem):
    pltpu.make_async_copy(view, view, sem).wait()


def _lane_tiles(x):
    return [x[:, c:c + DH] for c in range(0, x.shape[1], DH)]


def _own_rows(parts):
    row = lax.broadcasted_iota(jnp.int32, parts[0].shape, 0)
    out = parts[0]
    for h in range(1, len(parts)):
        out = jnp.where(row == h, parts[h], out)
    return out


def _kernel(ax, ak, av, awq, awo, bx, bk, bv, bwq, bwo, o_ref,
            x_buf, wq_buf, wo_buf, ring, q_scr, s_scr, m_scr, l_scr, acc_scr, out_scr,
            ring_sem, w_sem, tail_sem):
    dtype = ring.dtype

    def start_weights(lo, hi):
        @pl.loop(lo, hi)
        def _(n):
            col_blocks = H * DH // WQ_COLS
            wq_rows = _block(n >> _log2(col_blocks), WQ_ROWS)
            wq_cols = _block(n & (col_blocks - 1), WQ_COLS)
            wo_rows = _block(n, WO_ROWS)
            for matrix, j, first, count, priority in W_COPIES:
                if matrix == "wq":
                    copy = pltpu.make_async_copy(
                        (awq, bwq)[j].at[pl.ds(first, count), wq_rows, wq_cols],
                        wq_buf.at[j, pl.ds(first, count), wq_rows, wq_cols],
                        w_sem.at[0])
                else:
                    copy = pltpu.make_async_copy(
                        (awo, bwo)[j].at[pl.ds(first, count), wo_rows],
                        wo_buf.at[pl.ds(WQ * j + first, count), wo_rows],
                        w_sem.at[1])
                copy.start(priority=priority)

    def tail_copy(k):
        rows = pl.ds(TAIL[k][0], TAIL[k][1] - TAIL[k][0])
        return pltpu.make_async_copy(
            bwo.at[WQ - 1, rows], wo_buf.at[NG - 1, rows], tail_sem.at[k])

    def start_step(cache, t):
        slot = t & (SLOTS - 1)
        head0 = (t >> _log2(NKB)) * GH
        round0 = (t & (NKB - 1)) * (KB // KV_KEYS)

        @pl.loop(0, KB // KV_KEYS)
        def _(i):
            for head, priority in KV_COPIES:
                pltpu.make_async_copy(
                    cache.at[0, pl.ds(head0 + head, 2), _block(round0 + i, KV_KEYS)],
                    ring.at[slot, pl.ds(head, 2), _block(i, KV_KEYS)],
                    ring_sem.at[slot],
                ).start(priority=priority)

    def start_ahead(t, caches):
        n = t + LAG
        for i, cache in enumerate(caches):
            @pl.when((n >> _log2(NS)) == i)
            def _():
                start_step(cache, n & (NS - 1))

    def project_q(t):
        j = t >> _log2(NS)
        g0 = ((t & (NS - 1)) >> _log2(NKB)) * 2
        x = jnp.broadcast_to(x_buf[j, 0], (G, D))
        for u in range(2):
            w = wq_buf[j, :, :, _block(g0 + u, G * DH)].reshape(D, G * DH)
            q = jnp.dot(x, w, preferred_element_type=jnp.float32)
            q_scr[u] = _own_rows(_lane_tiles(q))

    def scores(t):
        slot = t & (SLOTS - 1)
        g0 = (t >> _log2(NKB)) * 2
        _wait_all(ring.at[slot], ring_sem.at[slot])
        for u in range(2):
            q = q_scr[u].astype(dtype)
            s = _own_rows([
                lax.dot_general(q, ring[slot, u * G + h], (((1,), (1,)), ((), ())),
                                preferred_element_type=jnp.float32)
                for h in range(G)
            ]) * (DH ** -0.5)
            s_scr[t, u] = s
            m = m_scr[g0 + u]
            for tile in _lane_tiles(s):
                m = jnp.maximum(m, tile)
            m_scr[g0 + u] = m

    def values(t):
        slot = t & (SLOTS - 1)
        g0 = (t >> _log2(NKB)) * 2
        probs = []
        for u in range(2):
            row_max = jnp.max(m_scr[g0 + u], axis=-1, keepdims=True)
            p = jnp.exp(s_scr[t, u] - row_max)
            l = l_scr[g0 + u]
            for tile in _lane_tiles(p):
                l = l + tile
            l_scr[g0 + u] = l
            probs.append(p.astype(dtype))
        _wait_all(ring.at[slot], ring_sem.at[slot])
        for u in range(2):
            acc_scr[g0 + u] += _own_rows([
                jnp.dot(probs[u], ring[slot, u * G + h], preferred_element_type=jnp.float32)
                for h in range(G)
            ])

    def head_outputs(g):
        o = acc_scr[g] / jnp.sum(l_scr[g], axis=-1, keepdims=True)
        return [jnp.broadcast_to(o[h:h + 1], (G, DH)).astype(dtype) for h in range(G)]

    start_weights(0, 4)
    x_copies = [pltpu.make_async_copy(x, x_buf.at[j], w_sem.at[2 + j])
                for j, x in enumerate((ax, bx))]
    for c in x_copies:
        c.start()
    m_scr[...] = jnp.full(m_scr.shape, -jnp.inf, jnp.float32)
    l_scr[...] = jnp.zeros(l_scr.shape, jnp.float32)
    acc_scr[...] = jnp.zeros(acc_scr.shape, jnp.float32)
    out_scr[...] = jnp.zeros(out_scr.shape, jnp.float32)
    start_weights(4, W_ROUNDS)

    @pl.loop(0, LAG)
    def _(t):
        start_step(ak, t)

    for c in x_copies:
        c.wait()
    _wait_all(wq_buf, w_sem.at[0])
    _wait_all(wo_buf.at[pl.ds(0, NG - 1)], w_sem.at[1])

    @pl.loop(0, 2 * NS)
    def _(t):
        @pl.when((t & (NKB - 1)) == 0)
        def _():
            project_q(t)

        start_ahead(t, (ak, bk, av))
        scores(t)

    @pl.loop(0, 2 * NS)
    def _(t):
        start_ahead(t, (av, bv))

        @pl.when(t + LAG == 2 * NS)
        def _():
            for k in range(len(TAIL)):
                tail_copy(k).start(priority=1)

        values(t)

        @pl.when(jnp.logical_and(((t + 1) & (NKB - 1)) < 2, t > 0))
        def _():
            g = 2 * (((t + 1) >> _log2(NKB)) - 1) + ((t + 1) & 1)
            out_scr[g >> _log2(NG // 2)] += jnp.dot(
                jnp.concatenate(head_outputs(g), axis=1), wo_buf[g],
                preferred_element_type=jnp.float32)

    o_ref[0, :, pl.ds(0, D)] = out_scr[0, 0:1].astype(o_ref.dtype)

    heads = head_outputs(NG - 1)
    split = TAIL[0][1]
    column = jnp.concatenate([
        jnp.broadcast_to(head[0:1].astype(jnp.float32), (DH, DH)).T
        for head in heads[split // DH:]
    ], axis=0)
    tail_copy(0).wait()
    out = out_scr[1] + jnp.dot(
        jnp.concatenate(heads[:split // DH], axis=1), wo_buf[NG - 1, pl.ds(0, split)],
        preferred_element_type=jnp.float32)
    out = jnp.where(lax.broadcasted_iota(jnp.int32, out.shape, 0) == 0, out, 0.0)
    for k, (lo, hi) in enumerate(TAIL):
        if k:
            tail_copy(k).wait()
            w = wo_buf[NG - 1, pl.ds(lo, hi - lo)].astype(jnp.float32)
            w = w * jnp.concatenate([column[lo - split:hi - split]] * (D // DH), axis=1)
            out += jnp.sum(w.reshape((hi - lo) // G, G, D), axis=0)
    o_ref[0, :, pl.ds(D, D)] = jnp.sum(out, axis=0, keepdims=True).astype(o_ref.dtype)


@jax.jit
def pallas_concat_heads__mha_block_cached__gqa_block_cached__decode_kernel(
    A_x: jax.Array,
    A_k_cache: jax.Array,
    A_v_cache: jax.Array,
    A_wq: jax.Array,
    A_wo: jax.Array,
    B_x: jax.Array,
    B_k_cache: jax.Array,
    B_v_cache: jax.Array,
    B_wq: jax.Array,
    B_wo: jax.Array,
):
    for cache in (A_k_cache, A_v_cache, B_k_cache, B_v_cache):
        assert cache.shape == (1, H, S, DH), cache.shape
    dtype = A_k_cache.dtype
    split_wq = lambda w: w.reshape(WQ, D // WQ, H * DH)
    split_wo = lambda w: w.reshape(WQ, H * DH // WQ, D)

    return pl.pallas_call(
        _kernel,
        out_shape=jax.ShapeDtypeStruct((1, 1, 2 * D), A_x.dtype),
        in_specs=[pl.BlockSpec(memory_space=pl.ANY)] * 10,
        out_specs=pl.BlockSpec(memory_space=pltpu.VMEM),
        scratch_shapes=[
            pltpu.VMEM((2, 1, 1, D), dtype),
            pltpu.VMEM((2, WQ, D // WQ, H * DH), dtype),
            pltpu.VMEM((NG, G * DH, D), dtype),
            pltpu.VMEM((SLOTS, GH, KB, DH), dtype),
            pltpu.VMEM((2, G, DH), jnp.float32),
            pltpu.VMEM((2 * NS, 2, G, KB), jnp.float32),
            pltpu.VMEM((NG, G, DH), jnp.float32),
            pltpu.VMEM((NG, G, DH), jnp.float32),
            pltpu.VMEM((NG, G, DH), jnp.float32),
            pltpu.VMEM((2, G, D), jnp.float32),
            pltpu.SemaphoreType.DMA((SLOTS,)),
            pltpu.SemaphoreType.DMA((4,)),
            pltpu.SemaphoreType.DMA((len(TAIL),)),
        ],
        compiler_params=pltpu.CompilerParams(
            vmem_limit_bytes=48 * 1024 * 1024,
            disable_semaphore_checks=True,
        ),
    )(A_x, A_k_cache, A_v_cache, split_wq(A_wq), split_wo(A_wo),
      B_x, B_k_cache, B_v_cache, split_wq(B_wq), split_wo(B_wo))
```
